```python
import os as _os
_os.environ.setdefault("JAX_PLATFORMS", "cpu")
import jax
import jax.numpy as jnp

def _softmax(x, axis=-1):
    return jax.nn.softmax(x, axis=axis)
def _gelu(x):
    return jax.nn.gelu(x, approximate=True)
def _silu(x):
    return jax.nn.silu(x)
def _sigmoid(x):
    return jax.nn.sigmoid(x)
def _layernorm(x, axis=-1, eps=1e-5):
    m = jnp.mean(x, axis=axis, keepdims=True)
    v = jnp.var(x, axis=axis, keepdims=True)
    return (x - m) / jnp.sqrt(v + eps)
def _scatter_add(tgt, idx, src, axis=0):
    return tgt.at[idx].add(src)
def _segment_sum(src, seg, n):
    return jax.ops.segment_sum(src, seg, n)
class _Rng:
    def __init__(self, key):
        self._k = key
    def _next(self):
        self._k, sub = jax.random.split(self._k)
        return sub
    def normal(self, shape):
        return jax.random.normal(self._next(), shape, dtype=jnp.bfloat16)
    def randint(self, lo, hi, shape):
        return jax.random.randint(self._next(), shape, lo, hi, dtype=jnp.int32)
    def uniform(self, shape, lo=0.0, hi=1.0):
        return jax.random.uniform(self._next(), shape, jnp.bfloat16, lo, hi)
    def permutation(self, n):
        return jax.random.permutation(self._next(), n)


kernel_name = 'concat_heads__gqa_block_cached__gqa_block_cached__near_ridge'

def setup_inputs():
    _rng = _Rng(jax.random.key(int.from_bytes(__import__("os").urandom(4), "little")))
    _w = (lambda a: (lambda t: t.astype(jnp.bfloat16) if jnp.issubdtype(t.dtype, jnp.floating) else t)(jnp.asarray(a)))
    def _A_setup():
        B, Sq, D = 8, 240, 640
        Hq, Hkv, Sk, Dh = 32, 32, 1024, 192
        assert Hq % Hkv == 0, (Hq, Hkv)
        return {
            "x": _w((lambda *s: _rng.normal(s) * 0.8)(B, Sq, D)),
            "k_cache": _w((lambda *s: _rng.normal(s) * 0.8)(B, Hkv, Sk, Dh)),
            "v_cache": _w((lambda *s: _rng.normal(s) * 0.05)(B, Hkv, Sk, Dh)),
            "wq": _w((lambda *s: _rng.normal(s) * 0.8)(D, Hq * Dh) * (D ** -0.5)),
            "wo": _w((lambda *s: _rng.normal(s) * 0.05)(Hq * Dh, D) * ((Hq * Dh) ** -0.5)),
        }
    _A_in = _A_setup()

    def _B_setup():
        B, Sq, D = 8, 240, 640
        Hq, Hkv, Sk, Dh = 32, 32, 1024, 192
        assert Hq % Hkv == 0, (Hq, Hkv)
        return {
            "x": _w((lambda *s: _rng.normal(s) * 0.8)(B, Sq, D)),
            "k_cache": _w((lambda *s: _rng.normal(s) * 0.8)(B, Hkv, Sk, Dh)),
            "v_cache": _w((lambda *s: _rng.normal(s) * 0.05)(B, Hkv, Sk, Dh)),
            "wq": _w((lambda *s: _rng.normal(s) * 0.8)(D, Hq * Dh) * (D ** -0.5)),
            "wo": _w((lambda *s: _rng.normal(s) * 0.05)(Hq * Dh, D) * ((Hq * Dh) ** -0.5)),
        }
    _B_in = _B_setup()

    return {
        "A_x": _A_in["x"],
        "A_k_cache": _A_in["k_cache"],
        "A_v_cache": _A_in["v_cache"],
        "A_wq": _A_in["wq"],
        "A_wo": _A_in["wo"],
        "B_x": _B_in["x"],
        "B_k_cache": _B_in["k_cache"],
        "B_v_cache": _B_in["v_cache"],
        "B_wq": _B_in["wq"],
        "B_wo": _B_in["wo"],
    }

def reference(A_x, A_k_cache, A_v_cache, A_wq, A_wo, B_x, B_k_cache, B_v_cache, B_wq, B_wo):
    def _A_ref(x, k_cache, v_cache, wq, wo):
        B, Sq, D = x.shape
        Hq, Dh = 32, 192
        Hkv = k_cache.shape[1]
        rep = Hq // Hkv
        q = (lambda x, *d: x.transpose(*d))((x @ wq).reshape(B, Sq, Hq, Dh), 0, 2, 1, 3)
        k = jnp.repeat(k_cache, rep, axis=1)
        v = jnp.repeat(v_cache, rep, axis=1)
        scores = jnp.einsum("bhqd,bhkd->bhqk", q, k) * (Dh ** -0.5)
        p = _softmax(scores, axis=-1)
        o = jnp.einsum("bhqk,bhkd->bhqd", p, v)
        return (lambda x, *d: x.transpose(*d))(o, 0, 2, 1, 3).reshape(B, Sq, Hq * Dh) @ wo

    def _B_ref(x, k_cache, v_cache, wq, wo):
        B, Sq, D = x.shape
        Hq, Dh = 32, 192
        Hkv = k_cache.shape[1]
        rep = Hq // Hkv
        q = (lambda x, *d: x.transpose(*d))((x @ wq).reshape(B, Sq, Hq, Dh), 0, 2, 1, 3)
        k = jnp.repeat(k_cache, rep, axis=1)
        v = jnp.repeat(v_cache, rep, axis=1)
        scores = jnp.einsum("bhqd,bhkd->bhqk", q, k) * (Dh ** -0.5)
        p = _softmax(scores, axis=-1)
        o = jnp.einsum("bhqk,bhkd->bhqd", p, v)
        return (lambda x, *d: x.transpose(*d))(o, 0, 2, 1, 3).reshape(B, Sq, Hq * Dh) @ wo

    a = _A_ref(A_x, A_k_cache, A_v_cache, A_wq, A_wo)
    b = _B_ref(B_x, B_k_cache, B_v_cache, B_wq, B_wo)
    return jnp.concatenate([a, b], axis=-1)
```

```python
import functools

import jax
import jax.numpy as jnp
import jax.experimental.pallas as pl
import jax.experimental.pallas.tpu as pltpu

HG = 4


def _attn_step(x_ref, k_ref, v_ref, wq_ref, wo_ref, o_ref, acc_ref, *, g, ng,
               dh, scale):
    hg = k_ref.shape[1]
    w = hg * dh
    col = pl.multiple_of(g * w, 128)

    x = x_ref[0]
    qg = jnp.dot(x, wq_ref[:, pl.ds(col, w)],
                 preferred_element_type=jnp.float32).astype(jnp.bfloat16)
    outs = []
    for h in range(hg):
        q = qg[:, h * dh:(h + 1) * dh]
        k = k_ref[0, h]
        v = v_ref[0, h]
        s = jax.lax.dot_general(q, k, (((1,), (1,)), ((), ())),
                                preferred_element_type=jnp.float32) * scale
        m = jnp.max(s, axis=-1, keepdims=True)
        p = jnp.exp(s - m)
        l = jnp.sum(p, axis=-1, keepdims=True)
        o = jnp.dot(p.astype(jnp.bfloat16), v,
                    preferred_element_type=jnp.float32)
        outs.append((o / l).astype(jnp.bfloat16))
    og = jnp.concatenate(outs, axis=-1)
    contrib = jnp.dot(og, wo_ref[pl.ds(col, w), :],
                      preferred_element_type=jnp.float32)

    @pl.when(g == 0)
    def _():
        acc_ref[...] = contrib

    @pl.when(g > 0)
    def _():
        acc_ref[...] += contrib

    @pl.when(g == ng - 1)
    def _():
        o_ref[0] = acc_ref[...].astype(o_ref.dtype)


def _kernel(ax_ref, ak_ref, av_ref, awq_ref, awo_ref,
            bx_ref, bk_ref, bv_ref, bwq_ref, bwo_ref,
            o_ref, acc_ref, *, ng, dh, scale):
    blk = pl.program_id(0)
    g = pl.program_id(2)

    @pl.when(blk == 0)
    def _():
        _attn_step(ax_ref, ak_ref, av_ref, awq_ref, awo_ref, o_ref, acc_ref,
                   g=g, ng=ng, dh=dh, scale=scale)

    @pl.when(blk == 1)
    def _():
        _attn_step(bx_ref, bk_ref, bv_ref, bwq_ref, bwo_ref, o_ref, acc_ref,
                   g=g, ng=ng, dh=dh, scale=scale)


@jax.jit
def pallas_concat_heads__gqa_block_cached__gqa_block_cached__near_ridge_kernel(
    A_x: jax.Array,
    A_k_cache: jax.Array,
    A_v_cache: jax.Array,
    A_wq: jax.Array,
    A_wo: jax.Array,
    B_x: jax.Array,
    B_k_cache: jax.Array,
    B_v_cache: jax.Array,
    B_wq: jax.Array,
    B_wo: jax.Array,
):
    B, Sq, D = A_x.shape
    _, Hkv, Sk, Dh = A_k_cache.shape
    Hq = A_wq.shape[1] // Dh
    assert Hq == Hkv
    assert Hq % HG == 0
    ng = Hq // HG
    scale = float(Dh) ** -0.5

    def a_x(blk, b, g):
        return (jnp.where(blk == 0, b, B - 1), 0, 0)

    def b_x(blk, b, g):
        return (jnp.where(blk == 1, b, 0), 0, 0)

    def a_kv(blk, b, g):
        return (jnp.where(blk == 0, b, B - 1), jnp.where(blk == 0, g, ng - 1), 0, 0)

    def b_kv(blk, b, g):
        return (jnp.where(blk == 1, b, 0), jnp.where(blk == 1, g, 0), 0, 0)

    const2 = lambda blk, b, g: (0, 0)
    one = pl.Buffered(1)

    def specs(x_map, kv_map):
        return [
            pl.BlockSpec((1, Sq, D), x_map),
            pl.BlockSpec((1, HG, Sk, Dh), kv_map),
            pl.BlockSpec((1, HG, Sk, Dh), kv_map),
            pl.BlockSpec((D, Hq * Dh), const2, pipeline_mode=one),
            pl.BlockSpec((Hq * Dh, D), const2, pipeline_mode=one),
        ]

    return pl.pallas_call(
        functools.partial(_kernel, ng=ng, dh=Dh, scale=scale),
        grid=(2, B, ng),
        in_specs=specs(a_x, a_kv) + specs(b_x, b_kv),
        out_specs=pl.BlockSpec((1, Sq, D), lambda blk, b, g: (b, 0, blk)),
        out_shape=jax.ShapeDtypeStruct((B, Sq, 2 * D), A_x.dtype),
        scratch_shapes=[pltpu.VMEM((Sq, D), jnp.float32)],
        compiler_params=pltpu.CompilerParams(
            dimension_semantics=("arbitrary", "arbitrary", "arbitrary"),
            vmem_limit_bytes=100 * 1024 * 1024,
        ),
    )(A_x, A_k_cache, A_v_cache, A_wq, A_wo,
      B_x, B_k_cache, B_v_cache, B_wq, B_wo)
```

```python
import functools
import math

import jax
import jax.numpy as jnp
import jax.experimental.pallas as pl
import jax.experimental.pallas.tpu as pltpu

HG = 8
AHEAD = 2


def _attn_step(x_ref, k_ref, v_ref, wq_ref, wo_ref, o_ref, acc_ref, *, g, ng,
               dh, scale):
    hg = k_ref.shape[1]
    c = scale * math.log2(math.e)

    x = x_ref[0]
    qg = jnp.dot(x, wq_ref[g],
                 preferred_element_type=jnp.float32).astype(jnp.bfloat16)

    def qk(h):
        q = qg[:, h * dh:(h + 1) * dh]
        return jnp.dot(q, k_ref[0, h],
                       preferred_element_type=jnp.float32)

    outs = []
    s_next = qk(0)
    for h in range(hg):
        s = s_next
        if h + 1 < hg:
            s_next = qk(h + 1)
        vt = v_ref[0, h]
        m = jnp.max(s, axis=-1, keepdims=True)
        p = jnp.exp2((s - m) * c)
        l = jnp.sum(p, axis=-1, keepdims=True)
        o = jax.lax.dot_general(p.astype(jnp.bfloat16), vt,
                                (((1,), (1,)), ((), ())),
                                preferred_element_type=jnp.float32)
        outs.append((o / l).astype(jnp.bfloat16))
    og = jnp.concatenate(outs, axis=-1)
    contrib = jnp.dot(og, wo_ref[g], preferred_element_type=jnp.float32)
    acc_ref[...] = jnp.where(g == 0, contrib, acc_ref[...] + contrib)

    @pl.when(g == ng - 1)
    def _():
        o_ref[0] = acc_ref[...].astype(o_ref.dtype)


def _kernel(ax_ref, ak_ref, av_ref, awq_hbm, awo_hbm,
            bx_ref, bk_ref, bv_ref, bwq_hbm, bwo_hbm,
            o_ref, acc_ref, wq_ref, wo_ref, sem, *, ng, dh, scale):
    blk = pl.program_id(0)
    b = pl.program_id(1)
    g = pl.program_id(2)
    w = wq_ref.shape[3]

    def copies(s, gg):
        wq_hbm, wo_hbm = ((awq_hbm, awo_hbm), (bwq_hbm, bwo_hbm))[s]
        return (
            pltpu.make_async_copy(wq_hbm.at[:, pl.ds(gg * w, w)],
                                  wq_ref.at[s, gg], sem.at[s, 0, gg]),
            pltpu.make_async_copy(wo_hbm.at[pl.ds(gg * w, w), :],
                                  wo_ref.at[s, gg], sem.at[s, 1, gg]),
        )

    first = (blk == 0) & (b == 0)

    @pl.when(first & (g == 0))
    def _():
        for gg in range(min(AHEAD, ng)):
            for cp in copies(0, gg):
                cp.start()

    for gg in range(ng):
        if gg + AHEAD < ng:
            @pl.when(first & (g == gg))
            def _():
                for cp in copies(0, gg + AHEAD):
                    cp.start()

        @pl.when((blk == 0) & (b == 1) & (g == gg))
        def _():
            for cp in copies(1, gg):
                cp.start()

    for s in range(2):
        for gg in range(ng):
            @pl.when((blk == s) & (b == 0) & (g == gg))
            def _():
                for cp in copies(s, gg):
                    cp.wait()

    @pl.when(blk == 0)
    def _():
        _attn_step(ax_ref, ak_ref, av_ref, wq_ref.at[0], wo_ref.at[0], o_ref,
                   acc_ref, g=g, ng=ng, dh=dh, scale=scale)

    @pl.when(blk == 1)
    def _():
        _attn_step(bx_ref, bk_ref, bv_ref, wq_ref.at[1], wo_ref.at[1], o_ref,
                   acc_ref, g=g, ng=ng, dh=dh, scale=scale)


@jax.jit
def pallas_concat_heads__gqa_block_cached__gqa_block_cached__near_ridge_kernel(
    A_x: jax.Array,
    A_k_cache: jax.Array,
    A_v_cache: jax.Array,
    A_wq: jax.Array,
    A_wo: jax.Array,
    B_x: jax.Array,
    B_k_cache: jax.Array,
    B_v_cache: jax.Array,
    B_wq: jax.Array,
    B_wo: jax.Array,
):
    B, Sq, D = A_x.shape
    _, Hkv, Sk, Dh = A_k_cache.shape
    Hq = A_wq.shape[1] // Dh
    assert Hq == Hkv and Hq % HG == 0 and B >= 2
    ng = Hq // HG
    scale = float(Dh) ** -0.5

    def a_x(blk, b, g):
        return (jnp.where(blk == 0, b, B - 1), 0, 0)

    def b_x(blk, b, g):
        return (jnp.where(blk == 1, b, 0), 0, 0)

    def a_kv(blk, b, g):
        return (jnp.where(blk == 0, b, B - 1), jnp.where(blk == 0, g, ng - 1), 0, 0)

    def b_kv(blk, b, g):
        return (jnp.where(blk == 1, b, 0), jnp.where(blk == 1, g, 0), 0, 0)

    def specs(x_map, kv_map):
        return [
            pl.BlockSpec((1, Sq, D), x_map),
            pl.BlockSpec((1, HG, Dh, Sk), kv_map),
            pl.BlockSpec((1, HG, Dh, Sk), kv_map),
            pl.BlockSpec(memory_space=pl.ANY),
            pl.BlockSpec(memory_space=pl.ANY),
        ]

    return pl.pallas_call(
        functools.partial(_kernel, ng=ng, dh=Dh, scale=scale),
        grid=(2, B, ng),
        in_specs=specs(a_x, a_kv) + specs(b_x, b_kv),
        out_specs=pl.BlockSpec((1, Sq, D), lambda blk, b, g: (b, 0, blk)),
        out_shape=jax.ShapeDtypeStruct((B, Sq, 2 * D), A_x.dtype),
        scratch_shapes=[pltpu.VMEM((Sq, D), jnp.float32),
                        pltpu.VMEM((2, ng, D, HG * Dh), jnp.bfloat16),
                        pltpu.VMEM((2, ng, HG * Dh, D), jnp.bfloat16),
                        pltpu.SemaphoreType.DMA((2, 2, ng))],
        compiler_params=pltpu.CompilerParams(
            dimension_semantics=("arbitrary", "arbitrary", "arbitrary"),
            vmem_limit_bytes=100 * 1024 * 1024,
        ),
    )(A_x, jnp.swapaxes(A_k_cache, 2, 3), jnp.swapaxes(A_v_cache, 2, 3), A_wq, A_wo,
      B_x, jnp.swapaxes(B_k_cache, 2, 3), jnp.swapaxes(B_v_cache, 2, 3), B_wq, B_wo)
```
